```python
import os as _os
_os.environ.setdefault("JAX_PLATFORMS", "cpu")
import jax
import jax.numpy as jnp

def _softmax(x, axis=-1):
    return jax.nn.softmax(x, axis=axis)
def _gelu(x):
    return jax.nn.gelu(x, approximate=True)
def _silu(x):
    return jax.nn.silu(x)
def _sigmoid(x):
    return jax.nn.sigmoid(x)
def _layernorm(x, axis=-1, eps=1e-5):
    m = jnp.mean(x, axis=axis, keepdims=True)
    v = jnp.var(x, axis=axis, keepdims=True)
    return (x - m) / jnp.sqrt(v + eps)
def _scatter_add(tgt, idx, src, axis=0):
    return tgt.at[idx].add(src)
def _segment_sum(src, seg, n):
    return jax.ops.segment_sum(src, seg, n)
class _Rng:
    def __init__(self, key):
        self._k = key
    def _next(self):
        self._k, sub = jax.random.split(self._k)
        return sub
    def normal(self, shape):
        return jax.random.normal(self._next(), shape, dtype=jnp.bfloat16)
    def randint(self, lo, hi, shape):
        return jax.random.randint(self._next(), shape, lo, hi, dtype=jnp.int32)
    def uniform(self, shape, lo=0.0, hi=1.0):
        return jax.random.uniform(self._next(), shape, jnp.bfloat16, lo, hi)
    def permutation(self, n):
        return jax.random.permutation(self._next(), n)


kernel_name = 'standalone__softmax_full_bidir__sampling'

def setup_inputs():
    _rng = _Rng(jax.random.key(int.from_bytes(__import__("os").urandom(4), "little")))
    _w = (lambda a: (lambda t: t.astype(jnp.bfloat16) if jnp.issubdtype(t.dtype, jnp.floating) else t)(jnp.asarray(a)))
    B, H, Sq, Skv, Dh = 8, 32, 1, 4096, 192
    return {
        "q": _w((lambda *s: _rng.normal(s) * 0.4)(B, H, Sq, Dh)),
        "k": _w((lambda *s: _rng.normal(s) * 0.4)(B, H, Skv, Dh)),
        "v": _w((lambda *s: _rng.normal(s) * 0.05)(B, H, Skv, Dh)),
    }

def reference(q, k, v):
    scale = q.shape[-1] ** -0.5
    scores = jnp.einsum('bhqd,bhkd->bhqk', q, k) * scale
    attn = _softmax(scores, axis=-1)
    return jnp.einsum('bhqk,bhkd->bhqd', attn, v)
```

```python
import jax
import jax.numpy as jnp
from jax import lax
import jax.experimental.pallas as pl
import jax.experimental.pallas.tpu as pltpu

_HEADS = 16
_ROWS = 8
_DEPTH = 4


@jax.jit
def pallas_standalone__softmax_full_bidir__sampling_kernel(
    q: jax.Array,
    k: jax.Array,
    v: jax.Array,
):
    B, H, SQ, D = q.shape
    S = k.shape[2]
    N = B * H
    assert SQ == 1 and N % _HEADS == 0 and D % _ROWS == 0 and S % 256 == 0
    n_groups = N // _HEADS
    n_steps = D // _ROWS
    assert n_steps >= _DEPTH
    half = _HEADS // 2
    width = _HEADS * _ROWS
    scale = D ** -0.5

    def kernel(q_hbm, k_hbm, v_hbm, o_hbm, buf, q_vm, o_vm, s_ref, p_ref, sems, io_sem):
        def start(src, g, r, slot):
            rows = pl.ds(pl.multiple_of(r * _ROWS, _ROWS), _ROWS)
            for h in range(half):
                for part in range(2):
                    cols = pl.ds(part * (S // 2), S // 2)
                    for prio in range(2):
                        hh = prio * half + h
                        pltpu.make_async_copy(
                            src.at[g * _HEADS + hh, rows, cols],
                            buf.at[slot, hh, :, cols],
                            sems.at[slot],
                        ).start(priority=prio)

        def wait(slot):
            pltpu.make_async_copy(buf.at[slot], buf.at[slot], sems.at[slot]).wait()

        def next_slot(slot):
            return jnp.where(slot + 1 == _DEPTH, 0, slot + 1)

        start(k_hbm, 0, 0, 0)
        q_copy = pltpu.make_async_copy(q_hbm, q_vm, io_sem)
        q_copy.start()
        lax.fori_loop(1, _DEPTH, lambda j, _: start(k_hbm, 0, j, j), None)
        q_copy.wait()

        row = lax.broadcasted_iota(jnp.int32, (_HEADS, width), 0)
        col = lax.broadcasted_iota(jnp.int32, (_HEADS, width), 1)
        own = (col // _ROWS) == row

        def group(g, slot):
            heads = pl.ds(pl.multiple_of(g * _HEADS, _HEADS), _HEADS)
            q_g = q_vm[heads, :]

            def k_step(r, slot):
                wait(slot)
                d_i = lax.broadcasted_iota(jnp.int32, (D, width), 0)
                c_i = lax.broadcasted_iota(jnp.int32, (D, width), 1)
                pick = (d_i == r * _ROWS + c_i % _ROWS).astype(q_g.dtype)
                q_r = jnp.dot(q_g, pick, preferred_element_type=jnp.float32)
                q_r = jnp.where(own, q_r, 0.0).astype(q_g.dtype)
                s_ref[...] += jnp.dot(q_r, buf[slot].reshape(width, S),
                                      preferred_element_type=jnp.float32)

                @pl.when(r + _DEPTH < n_steps)
                def _():
                    start(k_hbm, g, r + _DEPTH, slot)

                @pl.when(r + _DEPTH >= n_steps)
                def _():
                    start(v_hbm, g, r + _DEPTH - n_steps, slot)

                return next_slot(slot)

            s_ref[...] = jnp.zeros_like(s_ref)
            slot = lax.fori_loop(0, n_steps, k_step, slot)

            s = s_ref[...] * scale
            e = jnp.exp(s - jnp.max(s, axis=-1, keepdims=True))
            inv = 1.0 / jnp.sum(e, axis=-1, keepdims=True)
            p_ref[...] = e.astype(p_ref.dtype)

            def v_step(r, carry):
                slot, acc = carry
                wait(slot)
                o = lax.dot_general(p_ref[...], buf[slot].reshape(width, S),
                                    (((1,), (1,)), ((), ())),
                                    preferred_element_type=jnp.float32)
                o = jnp.where(own, o * inv, 0.0).astype(o_vm.dtype)
                c_i = lax.broadcasted_iota(jnp.int32, (width, D), 0)
                d_i = lax.broadcasted_iota(jnp.int32, (width, D), 1)
                place = (d_i == r * _ROWS + c_i % _ROWS).astype(o.dtype)
                acc = acc + jnp.dot(o, place, preferred_element_type=jnp.float32)

                @pl.when(r + _DEPTH < n_steps)
                def _():
                    start(v_hbm, g, r + _DEPTH, slot)

                @pl.when(jnp.logical_and(r + _DEPTH >= n_steps, g + 1 < n_groups))
                def _():
                    start(k_hbm, g + 1, r + _DEPTH - n_steps, slot)

                return next_slot(slot), acc

            slot, acc = lax.fori_loop(
                0, n_steps, v_step, (slot, jnp.zeros((_HEADS, D), jnp.float32)))
            o_vm[heads, :] = acc.astype(o_vm.dtype)
            return slot

        lax.fori_loop(0, n_groups, group, jnp.int32(0))
        o_copy = pltpu.make_async_copy(o_vm, o_hbm, io_sem)
        o_copy.start()
        o_copy.wait()

    out = pl.pallas_call(
        kernel,
        in_specs=[pl.BlockSpec(memory_space=pl.ANY)] * 3,
        out_specs=pl.BlockSpec(memory_space=pl.ANY),
        out_shape=jax.ShapeDtypeStruct((N, D), q.dtype),
        scratch_shapes=[
            pltpu.VMEM((_DEPTH, _HEADS, _ROWS, S), k.dtype),
            pltpu.VMEM((N, D), q.dtype),
            pltpu.VMEM((N, D), q.dtype),
            pltpu.VMEM((_HEADS, S), jnp.float32),
            pltpu.VMEM((_HEADS, S), v.dtype),
            pltpu.SemaphoreType.DMA((_DEPTH,)),
            pltpu.SemaphoreType.DMA(()),
        ],
    )(
        q.reshape(N, D),
        jnp.swapaxes(k, 2, 3).reshape(N, D, S),
        jnp.swapaxes(v, 2, 3).reshape(N, D, S),
    )
    return out.reshape(B, H, SQ, D)
```

```python
import jax
import jax.numpy as jnp
from jax import lax
import jax.experimental.pallas as pl
import jax.experimental.pallas.tpu as pltpu

_HEADS = 8
_ROWS = 8
_LANES = 2 * _HEADS * _ROWS
_DEPTH = 7


@jax.jit
def pallas_standalone__softmax_full_bidir__sampling_kernel(
    q: jax.Array,
    k: jax.Array,
    v: jax.Array,
):
    B, H, SQ, D = q.shape
    S = k.shape[2]
    N = B * H
    assert SQ == 1 and N % (2 * _HEADS) == 0 and N > 2 * _HEADS
    assert D % _ROWS == 0 and D // _ROWS >= _DEPTH and S % 256 == 0
    n_groups = N // _HEADS
    n_steps = D // _ROWS
    per_queue = _HEADS // 2
    blocks_per_vreg = _LANES // _ROWS
    half = S // 2
    scale = D**-0.5

    def kernel(q_hbm, k_hbm, v_hbm, o_hbm, buf, q_vm, o_vm, s_ref, p_ref, sems, io_sem):
        def before(t):
            return jnp.where(t == 0, n_steps - 1, t - 1)

        def position(part, head):
            return part * _HEADS + _HEADS - 1 - head

        def start_step(src, g, t, slot):
            rows = [
                pl.ds(pl.multiple_of(r * _ROWS, _ROWS), _ROWS) for r in (t, before(t))
            ]
            wrap = jnp.where(t == 0, 1, 0)
            queues = [[], []]
            for prio, queue in enumerate(queues):
                for h in range(per_queue):
                    queue.append((prio, 1, prio * per_queue + ((h - wrap) & (per_queue - 1))))
                    queue.append((prio, 0, prio * per_queue + h))
            order = [queues[1][0]]
            for pair in zip(queues[1][1:], queues[0]):
                order += pair
            order.append(queues[0][-1])
            for prio, part, head in order:
                pltpu.make_async_copy(
                    src.at[g * _HEADS + head, rows[part], pl.ds(part * half, half)],
                    buf.at[slot, position(part, head)],
                    sems.at[slot],
                ).start(priority=prio)

        def wait_step(slot):
            pltpu.make_async_copy(buf.at[slot], buf.at[slot], sems.at[slot]).wait()

        def next_slot(slot):
            return jnp.where(slot + 1 == _DEPTH, 0, slot + 1)

        def out_copy(first, count):
            rows = pl.ds(first, count)
            return pltpu.make_async_copy(o_vm.at[rows], o_hbm.at[rows], io_sem)

        q_copy = pltpu.make_async_copy(q_hbm, q_vm, io_sem)
        q_copy.start()
        lax.fori_loop(0, _DEPTH, lambda t, _: start_step(k_hbm, 0, t, t), None)
        q_copy.wait()

        early_rows = N - 2 * _HEADS
        early_out = out_copy(0, early_rows)
        late_out = out_copy(early_rows, N - early_rows)

        row = lax.broadcasted_iota(jnp.int32, (_HEADS, _LANES), 0)
        col = lax.broadcasted_iota(jnp.int32, (_HEADS, _LANES), 1)
        own = [col // _ROWS == position(part, row) for part in range(2)]

        def group(g, slot):
            heads = pl.ds(pl.multiple_of(g * _HEADS, _HEADS), _HEADS)
            q_g = q_vm[heads, :]

            def q_block(r):
                d = lax.broadcasted_iota(jnp.int32, (D, _LANES), 0)
                c = lax.broadcasted_iota(jnp.int32, (D, _LANES), 1)
                pick = (d == r * _ROWS + (c & (_ROWS - 1))).astype(q_g.dtype)
                return jnp.dot(q_g, pick, preferred_element_type=jnp.float32)

            def k_step(t, carry):
                slot, q_before = carry
                q_t = q_block(t)
                lhs = jnp.concatenate(
                    [jnp.where(own[0], q_t, 0.0), jnp.where(own[1], q_before, 0.0)]
                ).astype(q_g.dtype)
                wait_step(slot)
                s_ref[...] += jnp.dot(
                    lhs,
                    buf[slot].reshape(_LANES, half),
                    preferred_element_type=jnp.float32,
                )

                @pl.when(t + _DEPTH < n_steps)
                def _():
                    start_step(k_hbm, g, t + _DEPTH, slot)

                @pl.when(t + _DEPTH >= n_steps)
                def _():
                    start_step(v_hbm, g, t + _DEPTH - n_steps, slot)

                return next_slot(slot), q_t

            s_ref[...] = jnp.zeros_like(s_ref)
            slot, _ = lax.fori_loop(0, n_steps, k_step, (slot, q_block(n_steps - 1)))

            s = s_ref[...] * scale
            m = jnp.max(jnp.maximum(s[:_HEADS], s[_HEADS:]), axis=-1, keepdims=True)
            e = jnp.exp(s - jnp.concatenate([m, m]))
            inv_sum = 1.0 / jnp.sum(e[:_HEADS] + e[_HEADS:], axis=-1, keepdims=True)
            p_ref[...] = e.astype(p_ref.dtype)

            def diagonal(pv, part, r):
                x = jnp.where(own[part], pv[part * _HEADS : (part + 1) * _HEADS], 0.0)
                return x, ((r - position(part, 0)) * _ROWS + _LANES) & (_LANES - 1)

            def v_step(t, carry):
                slot, acc, pv_before = carry
                wait_step(slot)

                @pl.when(jnp.logical_and(t == n_steps - 1, g == n_groups - 1))
                def _():
                    early_out.start()

                pv = lax.dot_general(
                    p_ref[...],
                    buf[slot].reshape(_LANES, half),
                    (((1,), (1,)), ((), ())),
                    preferred_element_type=jnp.float32,
                )
                for part, r in ((1, before(before(t))), (0, before(t))):
                    x = pltpu.roll(*diagonal(pv_before, part, r), 1)
                    acc = [
                        a + jnp.where(r // blocks_per_vreg == i, x, 0.0)
                        for i, a in enumerate(acc)
                    ]

                @pl.when(t + _DEPTH < n_steps)
                def _():
                    start_step(v_hbm, g, t + _DEPTH, slot)

                @pl.when(jnp.logical_and(t + _DEPTH >= n_steps, g + 1 < n_groups))
                def _():
                    start_step(k_hbm, g + 1, t + _DEPTH - n_steps, slot)

                return next_slot(slot), acc, pv

            acc = [jnp.zeros((_HEADS, _LANES), jnp.float32)] * pl.cdiv(D, _LANES)
            pv = jnp.zeros((2 * _HEADS, _LANES), jnp.float32)
            slot, acc, pv = lax.fori_loop(0, n_steps, v_step, (slot, acc, pv))

            def unskew(x, shift):
                x = x * inv_sum
                if shift > _LANES // 2:
                    x, shift = pltpu.roll(x, shift, 1), 0
                return pltpu.roll(x, shift, 1, stride=_ROWS, stride_axis=0)

            out = [unskew(a, 0) for a in acc]
            for part, r in ((1, n_steps - 2), (0, n_steps - 1)):
                out[r // blocks_per_vreg] += unskew(*diagonal(pv, part, r))
            o_vm[heads, :] = jnp.concatenate(out, axis=1)[:, :D].astype(o_vm.dtype)
            return slot

        lax.fori_loop(0, n_groups, group, jnp.int32(0))
        late_out.start()
        early_out.wait()
        late_out.wait()

    out = pl.pallas_call(
        kernel,
        in_specs=[pl.BlockSpec(memory_space=pl.ANY)] * 3,
        out_specs=pl.BlockSpec(memory_space=pl.ANY),
        out_shape=jax.ShapeDtypeStruct((N, D), q.dtype),
        scratch_shapes=[
            pltpu.VMEM((_DEPTH, 2 * _HEADS, _ROWS, half), k.dtype),
            pltpu.VMEM((N, D), q.dtype),
            pltpu.VMEM((N, D), q.dtype),
            pltpu.VMEM((2 * _HEADS, half), jnp.float32),
            pltpu.VMEM((2 * _HEADS, half), v.dtype),
            pltpu.SemaphoreType.DMA((_DEPTH,)),
            pltpu.SemaphoreType.DMA(()),
        ],
    )(
        q.reshape(N, D),
        jnp.swapaxes(k, 2, 3).reshape(N, D, S),
        jnp.swapaxes(v, 2, 3).reshape(N, D, S),
    )
    return out.reshape(B, H, SQ, D)
```
